```python
import os as _os
_os.environ.setdefault("JAX_PLATFORMS", "cpu")
import jax
import jax.numpy as jnp

def _softmax(x, axis=-1):
    return jax.nn.softmax(x, axis=axis)
def _gelu(x):
    return jax.nn.gelu(x, approximate=True)
def _silu(x):
    return jax.nn.silu(x)
def _sigmoid(x):
    return jax.nn.sigmoid(x)
def _layernorm(x, axis=-1, eps=1e-5):
    m = jnp.mean(x, axis=axis, keepdims=True)
    v = jnp.var(x, axis=axis, keepdims=True)
    return (x - m) / jnp.sqrt(v + eps)
def _scatter_add(tgt, idx, src, axis=0):
    return tgt.at[idx].add(src)
def _segment_sum(src, seg, n):
    return jax.ops.segment_sum(src, seg, n)
class _Rng:
    def __init__(self, key):
        self._k = key
    def _next(self):
        self._k, sub = jax.random.split(self._k)
        return sub
    def normal(self, shape):
        return jax.random.normal(self._next(), shape, dtype=jnp.bfloat16)
    def randint(self, lo, hi, shape):
        return jax.random.randint(self._next(), shape, lo, hi, dtype=jnp.int32)
    def uniform(self, shape, lo=0.0, hi=1.0):
        return jax.random.uniform(self._next(), shape, jnp.bfloat16, lo, hi)
    def permutation(self, n):
        return jax.random.permutation(self._next(), n)


kernel_name = 'sequential_preLN__mha_block__dense_activation_mish__prompt'

def setup_inputs():
    _rng = _Rng(jax.random.key(int.from_bytes(__import__("os").urandom(4), "little")))
    _w = (lambda a: (lambda t: t.astype(jnp.bfloat16) if jnp.issubdtype(t.dtype, jnp.floating) else t)(jnp.asarray(a)))
    def _A_setup():
        B, S, D, H = 1, 2048, 576, 32
        return {
            "x": _w((lambda *s: _rng.normal(s) * 0.05)(B, S, D)),
            "wqkv": _w((lambda *s: _rng.normal(s) * 0.05)(D, 3 * D)),
            "wo": _w((lambda *s: _rng.normal(s) * 0.05)(D, D)),
        }
    _A_in = _A_setup()

    def _B_setup():
        B, S, D, F = 1, 2048, 576, 4608
        return {
            "x": _w((lambda *s: _rng.normal(s) * 0.05)(B, S, D)),
            "w1": _w((lambda *s: _rng.normal(s) * 1.6)(D, F) * (D ** -0.5)),
            "b1": _w((lambda *s: _rng.normal(s) * 0.05)(F)),
            "w2": _w((lambda *s: _rng.normal(s) * 0.05)(F, D) * (F ** -0.5)),
        }
    _B_in = _B_setup()

    return {
        "A_x": _A_in["x"],
        "A_wqkv": _A_in["wqkv"],
        "A_wo": _A_in["wo"],
        "B_x": _B_in["x"],
        "B_w1": _B_in["w1"],
        "B_b1": _B_in["b1"],
        "B_w2": _B_in["w2"],
    }

def reference(A_x, A_wqkv, A_wo, B_x, B_w1, B_b1, B_w2):
    def _A_ref(x, wqkv, wo):
        B, S, D = x.shape
        H = 32
        Dh = D // H
        qkv = (lambda x, *d: x.transpose(*d))((x @ wqkv).reshape(B, S, 3, H, Dh), 2, 0, 3, 1, 4)
        q, k, v = qkv[0], qkv[1], qkv[2]
        scores = jnp.einsum("bhqd,bhkd->bhqk", q, k) * (Dh ** -0.5)
        p = _softmax(scores, axis=-1)
        o = jnp.einsum("bhqk,bhkd->bhqd", p, v)
        return (lambda x, *d: x.transpose(*d))(o, 0, 2, 1, 3).reshape(B, S, D) @ wo

    def _B_ref(x, w1, b1, w2):
        h = jnp.einsum("bsd,df->bsf", x, w1) + b1
        sp = jnp.log1p(jnp.exp(-jnp.abs(h))) + jnp.where(h > 0, h, jnp.zeros_like(h))
        act = h * jnp.tanh(sp)
        return jnp.einsum("bsf,fd->bsd", act, w2)

    x = A_x
    h = x + _A_ref(_layernorm(x, axis=-1), A_wqkv, A_wo)
    h2 = h + _B_ref(_layernorm(h, axis=-1), B_w1, B_b1, B_w2)
    return h2
```

```python
import jax
import jax.numpy as jnp
import numpy as np
from jax import lax
import jax.experimental.pallas as pl
import jax.experimental.pallas.tpu as pltpu


S = 2048
D = 576
H = 32
DH = 18
F = 4608
NG = 5
HPG = 7
BQ = 512
CK = 128
U = 4
DELTA = 1
TB1 = 512
TB3 = 256
FC = 4608
LOG2E = 1.4426950408889634
EPS = 1e-5
NQ = S // BQ
NC = S // CK
WIN = 24
NT = (((1,), (1,)), ((), ()))
TN = (((0,), (0,)), ((), ()))


def _ln_t(xt):
    m = jnp.mean(xt, axis=0, keepdims=True)
    xc = xt - m
    v = jnp.mean(xc * xc, axis=0, keepdims=True)
    return xc * lax.rsqrt(v + EPS)


def _kernel(xt_hbm, wqkv_hbm, wo_hbm, w1_hbm, b1_hbm, w2t_hbm, out_hbm,
            xt_s, wqkv_s, wqk_s, wt_s, qt_s, k_s, vt_s, ot_s, s0_s, s1_s, qm_s,
            wo_s, wot_s, w1_s, b1_s, w2t_s, o_s, sems):
    cp_w = pltpu.make_async_copy(wqkv_hbm, wqkv_s, sems.at[0])
    cp_x = [pltpu.make_async_copy(xt_hbm.at[:, pl.ds(t * TB1, TB1)], xt_s.at[:, pl.ds(t * TB1, TB1)], sems.at[1 + t])
            for t in range(S // TB1)]
    nx = S // TB1
    cps = [pltpu.make_async_copy(wo_hbm, wo_s, sems.at[1 + nx]),
           pltpu.make_async_copy(w1_hbm, w1_s, sems.at[2 + nx]),
           pltpu.make_async_copy(b1_hbm, b1_s, sems.at[3 + nx]),
           pltpu.make_async_copy(w2t_hbm, w2t_s, sems.at[4 + nx])]
    cp_w.start()
    for c in cp_x:
        c.start()
    for c in cps:
        c.start()

    cp_w.wait()
    for g in range(NG):
        o = g * HPG * DH
        wt_s[g * 128:(g + 1) * 128, :] = wqkv_s[:, o:o + 128].T
        wqk_s[:, g * 128:(g + 1) * 128] = wqkv_s[:, D + o:D + o + 128]
    wt_s[NG * 128:, :] = wqkv_s[:, 2 * D:3 * D].T
    qscale = np.float32((DH ** -0.5) * LOG2E)

    for t in range(S // TB1):
        c0 = t * TB1
        cp_x[t].wait()
        xb = xt_s[:, c0:c0 + TB1].astype(jnp.float32)
        xn = _ln_t(xb).astype(jnp.bfloat16)
        qv = jnp.dot(wt_s[...], xn, preferred_element_type=jnp.float32)
        for g in range(NG):
            qt_s[g, :, c0:c0 + TB1] = pltpu.bitcast((qv[g * 128:(g + 1) * 128, :] * qscale).astype(jnp.bfloat16), jnp.uint32)
        vt_s[:, c0:c0 + TB1] = qv[NG * 128:, :].astype(jnp.bfloat16).astype(jnp.float32)
        kk = lax.dot_general(xn, wqk_s[...], TN, preferred_element_type=jnp.float32)
        for g in range(NG):
            k_s[g, c0 // 2:(c0 + TB1) // 2, :] = pltpu.bitcast(kk[:, g * 128:(g + 1) * 128].astype(jnp.bfloat16), jnp.uint32)

    rowq = lax.broadcasted_iota(jnp.int32, (64, BQ), 0)
    row = lax.broadcasted_iota(jnp.int32, (WIN, BQ), 0)
    rowv = lax.broadcasted_iota(jnp.int32, (WIN, CK), 0)
    sbuf = (s0_s, s1_s)
    LAG = NC + DELTA

    def run(base, nsteps, doA, bmin, state):
        mrun, mfin, acc = state
        mrun, mfin, acc = dict(mrun), dict(mfin), dict(acc)
        hinfo = {}

        def head_of(rel):
            if rel not in hinfo:
                it = base + rel
                hinfo[rel] = (it // NQ, it % NQ)
            return hinfo[rel]

        def qcols(qb):
            if isinstance(qb, int):
                return slice(qb * BQ, (qb + 1) * BQ)
            return pl.ds(pl.multiple_of(qb * BQ, BQ), BQ)

        for t in range(nsteps):
            if doA:
                ra, ca = divmod(t, NC)
                h, qb = head_of(ra)
                g = h // HPG
                if ca == 0:
                    j = h % HPG
                    q = qt_s[g, :, qcols(qb)]
                    qm_s[ra % U] = jnp.where((rowq >= j * (DH // 2)) & (rowq < (j + 1) * (DH // 2)), q, jnp.zeros_like(q))
                kc = pltpu.bitcast(k_s[g, ca * CK // 2:(ca + 1) * CK // 2, :], jnp.bfloat16)
                st = jnp.dot(kc, pltpu.bitcast(qm_s[ra % U], jnp.bfloat16), preferred_element_type=jnp.float32)
                sbuf[ra % 2][ca * CK:(ca + 1) * CK, :] = st
                mc = jnp.max(st.reshape(CK // 8, 8, BQ), axis=0)
                mrun[ra] = mc if ca == 0 else jnp.maximum(mrun[ra], mc)
            fb = t - LAG
            if fb >= bmin:
                rb, cb = divmod(fb, NC)
                hb, qbb = head_of(rb)
                win = (hb * DH // 8) * 8
                o = hb * DH - win
                r = (o + DH) % WIN
                if rb not in mfin:
                    mfin[rb] = jnp.max(mrun.pop(rb), axis=0, keepdims=True)
                p = jnp.exp2(sbuf[rb % 2][cb * CK:(cb + 1) * CK, :] - mfin[rb]).astype(jnp.bfloat16)
                vw = vt_s[pl.ds(pl.multiple_of(win, 8), WIN), cb * CK:(cb + 1) * CK]
                vw = jnp.where(rowv == r, jnp.ones_like(vw), vw)
                d = jnp.dot(vw, p, preferred_element_type=jnp.float32)
                acc[rb] = d if cb == 0 else acc[rb] + d
                if cb == NC - 1:
                    a = acc.pop(rb)
                    mfin.pop(rb)
                    l = jnp.sum(jnp.where(row == r, a, 0.0), axis=0, keepdims=True)
                    sl = (pl.ds(pl.multiple_of(win, 8), WIN), qcols(qbb))
                    old = ot_s[sl]
                    ot_s[sl] = jnp.where((row >= o) & (row < o + DH), a / l, old)
        return mrun, mfin, acc

    ot_s[...] = jnp.zeros_like(ot_s)
    assert U % 2 == 0 and 1 <= DELTA < NC
    NIT = H * NQ
    st0 = run(0, U * NC, True, 0, ({}, {}, {}))

    def shift(st):
        mrun, mfin, acc = st
        assert set(mrun) == {U - 1} and set(mfin) == {U - 2} and set(acc) == {U - 2}, (mrun.keys(), mfin.keys(), acc.keys())
        return mrun[U - 1], mfin[U - 2], acc[U - 2]

    def unshift(c):
        return {-1: c[0]}, {-2: c[1]}, {-2: c[2]}

    def body(i, c):
        base = i * U
        return shift(run(base, U * NC, True, -LAG, unshift(c)))

    c = lax.fori_loop(1, NIT // U, body, shift(st0))
    run(NIT, LAG, False, -LAG, unshift(c))

    for c in cps:
        c.wait()
    wot_s[...] = wo_s[...].T

    def p3_body(t, _):
        c0 = pl.multiple_of(t * TB3, TB3)
        ot = ot_s[:, pl.ds(c0, TB3)].astype(jnp.bfloat16)
        attn = jnp.dot(wot_s[...], ot, preferred_element_type=jnp.float32)
        h = xt_s[:, pl.ds(c0, TB3)].astype(jnp.float32) + attn
        hn = _ln_t(h).astype(jnp.bfloat16)
        y = h
        for fc in range(F // FC):
            z = lax.dot_general(hn, w1_s[:, fc * FC:(fc + 1) * FC], TN, preferred_element_type=jnp.float32)
            z = z + b1_s[:, fc * FC:(fc + 1) * FC].astype(jnp.float32)
            sp = jnp.log1p(jnp.exp(-jnp.abs(z))) + jnp.maximum(z, 0.0)
            act = (z * jnp.tanh(sp)).astype(jnp.bfloat16)
            y = y + lax.dot_general(w2t_s[:, fc * FC:(fc + 1) * FC], act, NT, preferred_element_type=jnp.float32)
        o_s[:, pl.ds(c0, TB3)] = y.astype(o_s.dtype)
        return 0

    lax.fori_loop(0, S // TB3, p3_body, 0)
    cp_o = pltpu.make_async_copy(o_s, out_hbm, sems.at[0])
    cp_o.start()
    cp_o.wait()


@jax.jit
def pallas_sequential_preLN__mha_block__dense_activation_mish__prompt_kernel(
    A_x, A_wqkv, A_wo, B_x, B_w1, B_b1, B_w2,
):
    del B_x
    xt = A_x.reshape(S, D).T
    w2t = B_w2.T
    b1 = B_b1.reshape(1, F)
    hbm = pl.BlockSpec(memory_space=pltpu.HBM)
    out_t = pl.pallas_call(
        _kernel,
        out_shape=jax.ShapeDtypeStruct((D, S), A_x.dtype),
        in_specs=[hbm] * 6,
        out_specs=hbm,
        scratch_shapes=[
            pltpu.VMEM((D, S), jnp.bfloat16),
            pltpu.VMEM((D, 3 * D), jnp.bfloat16),
            pltpu.VMEM((D, NG * 128), jnp.bfloat16),
            pltpu.VMEM((NG * 128 + D, D), jnp.bfloat16),
            pltpu.VMEM((NG, 64, S), jnp.uint32),
            pltpu.VMEM((NG, S // 2, 128), jnp.uint32),
            pltpu.VMEM((D, S), jnp.float32),
            pltpu.VMEM((D, S), jnp.float32),
            pltpu.VMEM((S, BQ), jnp.float32),
            pltpu.VMEM((S, BQ), jnp.float32),
            pltpu.VMEM((U, 64, BQ), jnp.uint32),
            pltpu.VMEM((D, D), jnp.bfloat16),
            pltpu.VMEM((D, D), jnp.bfloat16),
            pltpu.VMEM((D, F), jnp.bfloat16),
            pltpu.VMEM((1, F), jnp.bfloat16),
            pltpu.VMEM((D, F), jnp.bfloat16),
            pltpu.VMEM((D, S), jnp.bfloat16),
            pltpu.SemaphoreType.DMA((5 + S // TB1,)),
        ],
        compiler_params=pltpu.CompilerParams(vmem_limit_bytes=100 * 1024 * 1024),
    )(xt, A_wqkv, A_wo, B_w1, b1, w2t)
    return out_t.T.reshape(1, S, D)
```

```python
import jax
import jax.numpy as jnp
import numpy as np
from jax import lax
import jax.experimental.pallas as pl
import jax.experimental.pallas.tpu as pltpu

S = 2048
D = 576
H = 32
DH = 18
F = 4608
NG = 5
HPG = 7
BQ = 512
CK = 128
U = 8
DELTA = 1
TB1 = 512
TBA = 512
TB3 = 128
FC = 4608
LOG2E = 1.4426950408889634
EPS = 1e-5
NQ = S // BQ
NC = S // CK
WIN = 24
DEPSTEP = 18
QB0 = 2
QBN = 9
DEP = 1
QSPLIT = 0
VR = 8
MERGE = 1
MSTORE = 1
ORDER = 0
QPOS = 8
EPI_LAG = 0
QVLOOP = 0
KP = 640
NT = (((1,), (1,)), ((), ()))
TN = (((0,), (0,)), ((), ()))
BF = jnp.bfloat16
F32 = jnp.float32
U32 = jnp.uint32


def _ln_t(xt):
    m = jnp.mean(xt, axis=0, keepdims=True)
    xc = xt - m
    v = jnp.mean(xc * xc, axis=0, keepdims=True)
    return xc * lax.rsqrt(v + EPS)


def _kernel(xt_hbm, wqkv_hbm, wo_hbm, w1_hbm, b1_hbm, w2t_hbm, out_hbm,
            xt_s, wqkv_s, wk_s, wt_s, xn_s, xnn_s, qt_s, k_s, vt_s, ot_s, s0_s, s1_s, qm_s,
            wo_s, wot_s, w1_s, b1_s, w2t_s, hn_s, h_s, o_s, qh_s, qb_s, kb_s, sems):
    def wcopy(c0, c1, sem):
        return pltpu.make_async_copy(wqkv_hbm.at[:, pl.ds(c0, c1 - c0)], wqkv_s.at[:, pl.ds(c0, c1 - c0)], sem)

    def xcopy(c0, c1, sem):
        return pltpu.make_async_copy(xt_hbm.at[:, pl.ds(c0, c1 - c0)], xt_s.at[:, pl.ds(c0, c1 - c0)], sem)

    cp_wk = wcopy(512, 1280, sems.at[0])
    cp_x = [xcopy(t * TB1, (t + 1) * TB1, sems.at[9 + t]) for t in range(S // TB1)]
    cp_wq = wcopy(0, 512, sems.at[3])
    cp_wv = wcopy(1280, 3 * D, sems.at[4])
    cps = [pltpu.make_async_copy(wo_hbm, wo_s, sems.at[5]),
           pltpu.make_async_copy(w1_hbm, w1_s.at[pl.ds(0, D), :], sems.at[6]),
           pltpu.make_async_copy(b1_hbm, b1_s, sems.at[7]),
           pltpu.make_async_copy(w2t_hbm, w2t_s, sems.at[8])]
    for c in (cp_x[0], cp_wk, cp_x[1], cp_x[2], cp_wq, cp_wv, cp_x[3]):
        c.start()

    if MERGE:
        s1_s[...] = jnp.zeros_like(s1_s)
        s0_s[S - DELTA * CK:, :] = jnp.zeros((DELTA * CK, BQ), F32)
    qscale = np.float32((DH ** -0.5) * LOG2E)
    rowq = lax.broadcasted_iota(jnp.int32, (64, BQ), 0)
    assert TB1 == BQ
    nb = S // TB1
    assert nb == 4

    def ln1(t):
        c0 = t * TB1
        xn = _ln_t(xt_s[:, c0:c0 + TB1].astype(F32)).astype(BF)
        xn_s[:, c0:c0 + TB1] = xn
        xnn_s[c0:c0 + TB1, :] = xn.T

    def kproj(r0, r1):
        kk = jnp.dot(xnn_s[r0:r1, :], wk_s[...], preferred_element_type=F32)
        for g in range(NG):
            k_s[g, r0:r1, :] = kk[:, g * 128:(g + 1) * 128].astype(BF).astype(F32)

    HB = TB1 // 2
    with jax.named_scope("z0_wait_x0"):
        cp_x[0].wait()
    ln1(0)
    with jax.named_scope("z0b_wait_wk"):
        cp_wk.wait()
    for g in range(NG):
        o = g * HPG * DH
        wk_s[:, g * 128:(g + 1) * 128] = wqkv_s[:, D + o:D + o + 128]
    kproj(0, HB)
    with jax.named_scope("z0c_wait_x1"):
        cp_x[1].wait()
        cp_x[2].wait()
    ln1(1)
    kproj(HB, TB1)
    ln1(2)
    kproj(TB1, 2 * TB1)
    kproj(2 * TB1, 2 * TB1 + HB)
    with jax.named_scope("z0e_wait_rest"):
        cp_wq.wait()
        cp_wv.wait()
        cp_x[3].wait()
    ln1(3)
    kproj(2 * TB1 + HB, 3 * TB1)
    for g in range(NG):
        o = g * HPG * DH
        wt_s[g * 128:(g + 1) * 128, :] = wqkv_s[:, o:o + 128].T
    wt_s[NG * 128:, :] = wqkv_s[:, 2 * D:3 * D].T
    kproj(3 * TB1, 4 * TB1)

    def qvproj(t):
        if isinstance(t, int):
            cols = slice(t * TB1, (t + 1) * TB1)
        else:
            cols = pl.ds(pl.multiple_of(t * TB1, TB1), TB1)
        qv = jnp.dot(wt_s[...], xn_s[:, cols], preferred_element_type=F32)
        for g in range(NG):
            qg = (qv[g * 128:(g + 1) * 128, :] * qscale).astype(BF)
            qt_s[g, :, cols] = pltpu.bitcast(qg, U32)
            qf = qg.astype(F32)
            for j in range(HPG):
                h = g * HPG + j
                if h < H:
                    if VR:
                        qh_s[h, 0:DH, cols] = qf[j * DH:(j + 1) * DH, :]
        vt_s[:, cols] = qv[NG * 128:, :].astype(BF).astype(F32)

    if QVLOOP:
        qvproj(0)
        lax.fori_loop(1, nb, lambda t, _: qvproj(t), None)
    else:
        for t in range(nb):
            qvproj(t)

    row = lax.broadcasted_iota(jnp.int32, (WIN, BQ), 0)
    rowv = lax.broadcasted_iota(jnp.int32, (WIN, CK), 0)
    sbuf = (s0_s, s1_s)
    LAG = NC + DELTA
    NIT = H * NQ

    def qcols(qb):
        if isinstance(qb, int):
            return slice(qb * BQ, (qb + 1) * BQ)
        return pl.ds(pl.multiple_of(qb * BQ, BQ), BQ)

    row8 = lax.broadcasted_iota(jnp.int32, (8, BQ), 0)
    iota8 = lax.broadcasted_iota(jnp.int32, (8, 128), 0)

    def make_kb(h, slot, c, ds_):
        g = h // HPG
        j = h % HPG
        for v in range(VR // 8):
            kv = k_s[g, c * CK + CK - VR + v * 8:c * CK + CK - VR + v * 8 + 8, :]
            for d in ds_:
                idx = jnp.full((8, 128), d, jnp.int32) + j * DH
                kb_s[slot, c * (VR // 8) + v, d] = jnp.take_along_axis(kv, idx, axis=1)

    def qrow(h, d, qb):
        parts = []
        for i in range(BQ // 128):
            c = qb * BQ + i * 128
            cs = slice(c, c + 128) if isinstance(c, int) else pl.ds(pl.multiple_of(c, 128), 128)
            parts.append(jnp.broadcast_to(qh_s[h, d:d + 1, cs], (8, 128)))
        return jnp.concatenate(parts, axis=1)

    def make_qm(it, slot):
        h = it // NQ
        qb = it % NQ
        g = h // HPG
        j = h % HPG
        q = qt_s[g, :, qcols(qb)]
        qm_s[slot] = jnp.where((rowq >= j * (DH // 2)) & (rowq < (j + 1) * (DH // 2)), q, jnp.zeros_like(q))
        if VR:
            qa = qh_s[h, :, qcols(qb)]
            for d in range(DH):
                qb_s[slot, d] = jnp.broadcast_to(qa[d:d + 1, :], (8, BQ))

    def run(base, nsteps, doA, bmin, state, nextqm, trange=None):
        mrun, mfin, acc = state
        mrun, mfin, acc = dict(mrun), dict(mfin), dict(acc)
        hinfo = {}
        sthist = {}
        never = iota8 < -1 - base
        nxt = {}

        def head_of(rel):
            if rel not in hinfo:
                it = base + rel
                if MERGE and rel < 0 and not isinstance(it, int):
                    it = jnp.maximum(it, 0)
                hinfo[rel] = (it // NQ, it % NQ)
            return hinfo[rel]

        def stepA(t):
            ra, ca = divmod(t, NC)
            h, qb = head_of(ra)
            g = h // HPG
            MR = CK - VR
            st = jnp.dot(k_s[g, ca * CK:ca * CK + MR, :], pltpu.bitcast(qm_s[ra % U], BF), preferred_element_type=F32)
            sbuf[ra % 2][ca * CK:ca * CK + MR, :] = st
            mc = jnp.max(st.reshape(MR // 8, 8, BQ), axis=0)
            sthist[t] = st[MR - 8:MR, 0:128]
            for v0 in range(MR, CK, 8):
                sv = None
                for d in range(DH):
                    kb = kb_s[(ra // NQ) % 2, ca * (VR // 8) + (v0 - MR) // 8, d]
                    if DEP and (t - DEP) in sthist and d % DEPSTEP == 0:
                        kb = jnp.where(never, sthist[t - DEP], kb)
                    tt = jnp.concatenate([kb] * (BQ // 128), axis=1) * qb_s[ra % U, d]
                    sv = tt if sv is None else sv + tt
                sbuf[ra % 2][ca * CK + v0:ca * CK + v0 + 8, :] = sv
                mc = jnp.maximum(mc, sv)
            mrun[ra] = mc if ca == 0 else jnp.maximum(mrun[ra], mc)
            if VR:
                hn = h + 1
                hn = min(hn, H - 1) if isinstance(hn, int) else jnp.minimum(hn, H - 1)
                q4 = ra % NQ
                ds_ = range((q4 * DH) // NQ, ((q4 + 1) * DH) // NQ)
                make_kb(hn, (ra // NQ + 1) % 2, ca, ds_)

            if ca == QPOS and (ra < U - 1 or nextqm):
                it1 = base + ra + 1
                if ra == U - 1:
                    it1 = min(it1, NIT - 1) if isinstance(it1, int) else jnp.minimum(it1, NIT - 1)
                make_qm(it1, (ra + 1) % U)

        def stepB(t):
            fb = t - LAG
            rb, cb = divmod(fb, NC)
            hb, qbb = head_of(rb)
            win = (hb * DH // 8) * 8
            o = hb * DH - win
            r = (o + DH) % WIN
            if rb not in mfin:
                mfin[rb] = jnp.max(mrun.pop(rb), axis=0, keepdims=True)
            p = jnp.exp2(sbuf[rb % 2][cb * CK:(cb + 1) * CK, :] - mfin[rb]).astype(BF)
            wrows = pl.ds(pl.multiple_of(win, 8), WIN) if not isinstance(win, int) else slice(win, win + WIN)
            vw = vt_s[wrows, cb * CK:(cb + 1) * CK]
            vw = jnp.where(rowv == r, jnp.ones_like(vw), vw)
            d = jnp.dot(vw, p, preferred_element_type=F32)
            acc[rb] = d if cb == 0 else acc[rb] + d
            if cb == NC - 1:
                pend.append((t + EPI_LAG, rb, hb, qbb))
                mfin.pop(rb)

        def finish(t, force=False):
            for item in list(pend):
                if item[0] <= t or force:
                    pend.remove(item)
                    _, rb, hb_, qbb = item
                    ot_s[hb_, :, qcols(qbb)] = acc.pop(rb)

        pend = []
        for t in range(*(trange or (0, nsteps))):
            doB = t - LAG >= bmin
            if ORDER == 0:
                if doA:
                    stepA(t)
                if doB:
                    stepB(t)
            else:
                if doB:
                    stepB(t)
                if doA:
                    stepA(t)
            finish(t)
        finish(0, True)
        return mrun, mfin, acc

    assert U % 2 == 0 and 1 <= DELTA < NC
    make_qm(0, 0)
    if VR:
        for c in range(NC):
            make_kb(0, 0, c, range(DH))
    if not MERGE:
        st0 = run(0, U * NC, True, 0, ({}, {}, {}), True)

    def shift(st):
        mrun, mfin, acc = st
        assert set(mrun) == {U - 1} and set(mfin) == {U - 2} and set(acc) == {U - 2}, (mrun.keys(), mfin.keys(), acc.keys())
        return mrun[U - 1], mfin[U - 2], acc[U - 2]

    def unshift(c):
        return {-1: c[0]}, {-2: c[1]}, {-2: c[2]}

    def body(i, c):
        @pl.when(i == 2)
        def _():
            for cp in cps:
                cp.start()
        base = i * U
        return shift(run(base, U * NC, True, -LAG, unshift(c), True))

    with jax.named_scope("z3_attn_loop"):
        if MERGE:
            c0_ = (jnp.zeros((8, BQ), F32), jnp.zeros((1, BQ), F32), jnp.zeros((WIN, BQ), F32))
            c = lax.fori_loop(0, NIT // U, body, c0_)
        else:
            c = lax.fori_loop(1, NIT // U, body, shift(st0))
    for cp in cps:
        cp.wait()
    wot_s[...] = wo_s[...].T
    rowb = lax.broadcasted_iota(jnp.int32, (KP - D, 128), 0)
    for t in range(F // 128):
        brow = jnp.broadcast_to(b1_s[t:t + 1, :].astype(F32), (KP - D, 128))
        w1_s[D:, t * 128:(t + 1) * 128] = jnp.where(rowb == 0, brow, 0.0).astype(BF)

    ones_blk = (lax.broadcasted_iota(jnp.int32, (KP - D, TB3), 0) == 0).astype(F32)

    row8t = lax.broadcasted_iota(jnp.int32, (8, TB3), 0)

    def cols3(t):
        if isinstance(t, int):
            return slice(t * TB3, (t + 1) * TB3)
        return pl.ds(pl.multiple_of(t * TB3, TB3), TB3)

    def p3a(t, slot):
        cols = cols3(t)
        res = []
        for hh in range(H):
            win = (hh * DH // 8) * 8
            r = (hh * DH - win + DH) % WIN
            a = ot_s[hh, :, cols]
            res.append(a * pltpu.reciprocal(a[r:r + 1, :], full_range=False))
        blocks = []
        for v in range(D // 8):
            h0, h1 = (8 * v) // DH, (8 * v + 7) // DH
            w0 = (h0 * DH // 8) * 8
            blk = res[h0][8 * v - w0:8 * v - w0 + 8, :]
            if h1 != h0:
                w1 = (h1 * DH // 8) * 8
                blk = jnp.where(row8t < h1 * DH - 8 * v, blk, res[h1][8 * v - w1:8 * v - w1 + 8, :])
            blocks.append(blk)
        ot = jnp.concatenate(blocks, axis=0).astype(BF)
        attn = jnp.dot(wot_s[...], ot, preferred_element_type=F32)
        h = xt_s[:, cols].astype(F32) + attn
        h_s[slot] = h
        hn_s[slot] = jnp.concatenate([_ln_t(h), ones_blk], axis=0).astype(BF).T

    def ffn(t, slot):
        cols = cols3(t)
        hn = hn_s[slot]
        y = h_s[slot]
        for fc in range(F // FC):
            z = jnp.dot(hn, w1_s[:, fc * FC:(fc + 1) * FC], preferred_element_type=F32)
            sp = jnp.log1p(jnp.exp(-jnp.abs(z))) + jnp.maximum(z, 0.0)
            act = (z * jnp.tanh(sp)).astype(BF)
            y = y + lax.dot_general(w2t_s[:, fc * FC:(fc + 1) * FC], act, NT, preferred_element_type=F32)
        o_s[:, cols] = y.astype(o_s.dtype)

    st = unshift(c)
    for t in range(LAG):
        st = run(NIT, LAG, False, -LAG, st, False, (t, t + 1))
        if t == 0:
            p3a(0, 0)

    npair = S // (2 * TB3)

    def p3_body(i, _):
        t0 = 2 * i
        p3a(t0 + 1, 1)
        ffn(t0, 0)
        p3a(jnp.minimum(t0 + 2, S // TB3 - 1), 0)
        ffn(t0 + 1, 1)
        dcols = pl.ds(pl.multiple_of(t0 * TB3, 2 * TB3), 2 * TB3)
        pltpu.make_async_copy(o_s.at[:, dcols], out_hbm.at[:, dcols], sems.at[0]).start()
        return 0

    with jax.named_scope("z6_ffn_loop"):
        lax.fori_loop(0, npair, p3_body, 0)
    with jax.named_scope("z7_wait_out"):
        pltpu.make_async_copy(o_s, out_hbm, sems.at[0]).wait()


@jax.jit
def pallas_sequential_preLN__mha_block__dense_activation_mish__prompt_kernel(
    A_x, A_wqkv, A_wo, B_x, B_w1, B_b1, B_w2,
):
    del B_x
    xt = A_x.reshape(S, D).T
    w2t = B_w2.T
    b1 = B_b1.reshape(F // 128, 128)
    hbm = pl.BlockSpec(memory_space=pltpu.HBM)
    out_t = pl.pallas_call(
        _kernel,
        out_shape=jax.ShapeDtypeStruct((D, S), A_x.dtype),
        in_specs=[hbm] * 6,
        out_specs=hbm,
        scratch_shapes=[
            pltpu.VMEM((D, S), BF),
            pltpu.VMEM((D, 3 * D), BF),
            pltpu.VMEM((D, NG * 128), BF),
            pltpu.VMEM((NG * 128 + D, D), BF),
            pltpu.VMEM((D, S), BF),
            pltpu.VMEM((S, D), BF),
            pltpu.VMEM((NG, 64, S), U32),
            pltpu.VMEM((NG, S, 128), F32),
            pltpu.VMEM((D, S), F32),
            pltpu.VMEM((H, WIN, S), F32),
            pltpu.VMEM((S, BQ), F32),
            pltpu.VMEM((S, BQ), F32),
            pltpu.VMEM((U, 64, BQ), U32),
            pltpu.VMEM((D, D), BF),
            pltpu.VMEM((D, D), BF),
            pltpu.VMEM((KP, F), BF),
            pltpu.VMEM((F // 128, 128), BF),
            pltpu.VMEM((D, F), BF),
            pltpu.VMEM((2, TB3, KP), BF),
            pltpu.VMEM((2, D, TB3), F32),
            pltpu.VMEM((D, S), BF),
            pltpu.VMEM((H, WIN, S), F32),
            pltpu.VMEM((U, DH, 8, BQ), F32),
            pltpu.VMEM((2, NC * max(VR // 8, 1), DH, 8, 128), F32),
            pltpu.SemaphoreType.DMA((13,)),
        ],
        compiler_params=pltpu.CompilerParams(vmem_limit_bytes=120 * 1024 * 1024),
    )(xt, A_wqkv, A_wo, B_w1, b1, w2t)
    return out_t.T.reshape(1, S, D)
```

```python
import jax
import jax.numpy as jnp
import numpy as np
from jax import lax
import jax.experimental.pallas as pl
import jax.experimental.pallas.tpu as pltpu

S = 2048
D = 576
H = 32
DH = 18
F = 4608
NG = 5
HPG = 7
BQ = 512
CK = 128
U = 8
DELTA = 1
TB1 = 512
TBA = 512
TB3 = 128
FC = 4608
LOG2E = 1.4426950408889634
EPS = 1e-5
NQ = S // BQ
NC = S // CK
WIN = 24
DEPSTEP = 18
QB0 = 2
QBN = 9
DEP = 1
QSPLIT = 0
VR = 8
MERGE = 1
MSTORE = 1
ORDER = 0
QPOS = 8
EPI_LAG = 0
QVLOOP = 0
KP = 640
NT = (((1,), (1,)), ((), ()))
TN = (((0,), (0,)), ((), ()))
BF = jnp.bfloat16
F32 = jnp.float32
U32 = jnp.uint32


def _ln_t(xt):
    m = jnp.mean(xt, axis=0, keepdims=True)
    xc = xt - m
    v = jnp.mean(xc * xc, axis=0, keepdims=True)
    return xc * lax.rsqrt(v + EPS)


def _kernel(xt_hbm, wqkv_hbm, wo_hbm, w1_hbm, b1_hbm, w2t_hbm, out_hbm,
            xt_s, wqkv_s, wkt_s, wt_s, xn_s, qt_s, k_s, vt_s, ot_s, s0_s, s1_s, qm_s,
            wo_s, wot_s, w1_s, b1_s, w2t_s, hn_s, h_s, o_s, qh_s, qb_s, kb_s, sems):
    def wcopy(c0, c1, sem):
        return pltpu.make_async_copy(wqkv_hbm.at[:, pl.ds(c0, c1 - c0)], wqkv_s.at[:, pl.ds(c0, c1 - c0)], sem)

    def xcopy(c0, c1, sem):
        return pltpu.make_async_copy(xt_hbm.at[:, pl.ds(c0, c1 - c0)], xt_s.at[:, pl.ds(c0, c1 - c0)], sem)

    cp_wk = wcopy(512, 1280, sems.at[0])
    cp_x = [xcopy(t * TB1, (t + 1) * TB1, sems.at[9 + t]) for t in range(S // TB1)]
    cp_wq = wcopy(0, 512, sems.at[3])
    cp_wv = wcopy(1280, 3 * D, sems.at[4])
    cps = [pltpu.make_async_copy(wo_hbm, wo_s, sems.at[5]),
           pltpu.make_async_copy(w1_hbm, w1_s.at[pl.ds(0, D), :], sems.at[6]),
           pltpu.make_async_copy(b1_hbm, b1_s, sems.at[7]),
           pltpu.make_async_copy(w2t_hbm, w2t_s, sems.at[8])]
    for c in (cp_x[0], cp_wk, cp_x[1], cp_x[2], cp_wq, cp_wv, cp_x[3]):
        c.start()

    if MERGE:
        s1_s[...] = jnp.zeros_like(s1_s)
        s0_s[S - DELTA * CK:, :] = jnp.zeros((DELTA * CK, BQ), F32)
    qscale = np.float32((DH ** -0.5) * LOG2E)
    rowq = lax.broadcasted_iota(jnp.int32, (64, BQ), 0)
    assert TB1 == BQ
    nb = S // TB1
    assert nb == 4

    def ln1(t):
        c0 = t * TB1
        xn = _ln_t(xt_s[:, c0:c0 + TB1].astype(F32)).astype(BF)
        xn_s[:, c0:c0 + TB1] = xn

    def kproj(t, part=2):
        c0 = t * TB1
        lo, hi, gs = ((0, 256, (0, 1)), (240, D, (2, 3, 4)), (0, D, range(NG)))[part]
        kt = jnp.dot(wkt_s[lo:hi, :], xn_s[:, c0:c0 + TB1], preferred_element_type=F32).astype(BF)
        for g in gs:
            o = g * HPG * DH - lo
            blk = kt[o:min(o + 128, hi - lo), :]
            if blk.shape[0] < 128:
                blk = jnp.concatenate([blk, jnp.zeros((128 - blk.shape[0], TB1), BF)], axis=0)
            k_s[g, c0:c0 + TB1, :] = blk.T.astype(F32)

    with jax.named_scope("z0_wait_x0"):
        cp_x[0].wait()
    ln1(0)
    with jax.named_scope("z0b_wait_wk"):
        cp_wk.wait()
    wkt_s[...] = wqkv_s[:, D:2 * D].T
    kproj(0, 0)
    with jax.named_scope("z0c_wait_x1"):
        cp_x[1].wait()
        cp_x[2].wait()
    ln1(1)
    kproj(0, 1)
    ln1(2)
    kproj(1)
    kproj(2, 0)
    with jax.named_scope("z0e_wait_rest"):
        cp_wq.wait()
        cp_wv.wait()
        cp_x[3].wait()
    ln1(3)
    kproj(2, 1)
    wt_s[0:D, :] = wqkv_s[:, 0:D].T
    wt_s[D:, :] = wqkv_s[:, 2 * D:3 * D].T
    kproj(3)

    def qvproj(t):
        if isinstance(t, int):
            cols = slice(t * TB1, (t + 1) * TB1)
        else:
            cols = pl.ds(pl.multiple_of(t * TB1, TB1), TB1)
        qv = jnp.dot(wt_s[...], xn_s[:, cols], preferred_element_type=F32)
        qf = (qv[0:D + 64, :] * qscale).astype(BF)
        for g in range(NG):
            o = g * HPG * DH
            qt_s[g, :, cols] = pltpu.bitcast(qf[o:o + 128, :], U32)
        if VR:
            qf = qf.astype(F32)
            for h in range(H):
                qh_s[h, 0:DH, cols] = qf[h * DH:(h + 1) * DH, :]
        vt_s[:, cols] = qv[D:, :].astype(BF).astype(F32)

    if QVLOOP:
        qvproj(0)
        lax.fori_loop(1, nb, lambda t, _: qvproj(t), None)
    else:
        for t in range(nb):
            qvproj(t)

    row = lax.broadcasted_iota(jnp.int32, (WIN, BQ), 0)
    rowv = lax.broadcasted_iota(jnp.int32, (WIN, CK), 0)
    sbuf = (s0_s, s1_s)
    LAG = NC + DELTA
    NIT = H * NQ

    def qcols(qb):
        if isinstance(qb, int):
            return slice(qb * BQ, (qb + 1) * BQ)
        return pl.ds(pl.multiple_of(qb * BQ, BQ), BQ)

    row8 = lax.broadcasted_iota(jnp.int32, (8, BQ), 0)
    iota8 = lax.broadcasted_iota(jnp.int32, (8, 128), 0)

    def make_kb(h, slot, c, ds_):
        g = h // HPG
        j = h % HPG
        for v in range(VR // 8):
            kv = k_s[g, c * CK + CK - VR + v * 8:c * CK + CK - VR + v * 8 + 8, :]
            for d in ds_:
                idx = jnp.full((8, 128), d, jnp.int32) + j * DH
                kb_s[slot, c * (VR // 8) + v, d] = jnp.take_along_axis(kv, idx, axis=1)

    def qrow(h, d, qb):
        parts = []
        for i in range(BQ // 128):
            c = qb * BQ + i * 128
            cs = slice(c, c + 128) if isinstance(c, int) else pl.ds(pl.multiple_of(c, 128), 128)
            parts.append(jnp.broadcast_to(qh_s[h, d:d + 1, cs], (8, 128)))
        return jnp.concatenate(parts, axis=1)

    def make_qm(it, slot):
        h = it // NQ
        qb = it % NQ
        g = h // HPG
        j = h % HPG
        q = qt_s[g, :, qcols(qb)]
        qm_s[slot] = jnp.where((rowq >= j * (DH // 2)) & (rowq < (j + 1) * (DH // 2)), q, jnp.zeros_like(q))
        if VR:
            qa = qh_s[h, :, qcols(qb)]
            for d in range(DH):
                qb_s[slot, d] = jnp.broadcast_to(qa[d:d + 1, :], (8, BQ))

    def run(base, nsteps, doA, bmin, state, nextqm, trange=None):
        mrun, mfin, acc = state
        mrun, mfin, acc = dict(mrun), dict(mfin), dict(acc)
        hinfo = {}
        sthist = {}
        never = iota8 < -1 - base
        nxt = {}

        def head_of(rel):
            if rel not in hinfo:
                it = base + rel
                if MERGE and rel < 0 and not isinstance(it, int):
                    it = jnp.maximum(it, 0)
                hinfo[rel] = (it // NQ, it % NQ)
            return hinfo[rel]

        def stepA(t):
            ra, ca = divmod(t, NC)
            h, qb = head_of(ra)
            g = h // HPG
            MR = CK - VR
            st = jnp.dot(k_s[g, ca * CK:ca * CK + MR, :], pltpu.bitcast(qm_s[ra % U], BF), preferred_element_type=F32)
            sbuf[ra % 2][ca * CK:ca * CK + MR, :] = st
            mc = jnp.max(st.reshape(MR // 8, 8, BQ), axis=0)
            sthist[t] = st[MR - 8:MR, 0:128]
            for v0 in range(MR, CK, 8):
                sv = None
                for d in range(DH):
                    kb = kb_s[(ra // NQ) % 2, ca * (VR // 8) + (v0 - MR) // 8, d]
                    if DEP and (t - DEP) in sthist and d % DEPSTEP == 0:
                        kb = jnp.where(never, sthist[t - DEP], kb)
                    tt = jnp.concatenate([kb] * (BQ // 128), axis=1) * qb_s[ra % U, d]
                    sv = tt if sv is None else sv + tt
                sbuf[ra % 2][ca * CK + v0:ca * CK + v0 + 8, :] = sv
                mc = jnp.maximum(mc, sv)
            mrun[ra] = mc if ca == 0 else jnp.maximum(mrun[ra], mc)
            if VR:
                hn = h + 1
                hn = min(hn, H - 1) if isinstance(hn, int) else jnp.minimum(hn, H - 1)
                q4 = ra % NQ
                ds_ = range((q4 * DH) // NQ, ((q4 + 1) * DH) // NQ)
                make_kb(hn, (ra // NQ + 1) % 2, ca, ds_)

            if ca == QPOS and (ra < U - 1 or nextqm):
                it1 = base + ra + 1
                if ra == U - 1:
                    it1 = min(it1, NIT - 1) if isinstance(it1, int) else jnp.minimum(it1, NIT - 1)
                make_qm(it1, (ra + 1) % U)

        def stepB(t):
            fb = t - LAG
            rb, cb = divmod(fb, NC)
            hb, qbb = head_of(rb)
            win = (hb * DH // 8) * 8
            o = hb * DH - win
            r = (o + DH) % WIN
            if rb not in mfin:
                mfin[rb] = jnp.max(mrun.pop(rb), axis=0, keepdims=True)
            p = jnp.exp2(sbuf[rb % 2][cb * CK:(cb + 1) * CK, :] - mfin[rb]).astype(BF)
            wrows = pl.ds(pl.multiple_of(win, 8), WIN) if not isinstance(win, int) else slice(win, win + WIN)
            vw = vt_s[wrows, cb * CK:(cb + 1) * CK]
            vw = jnp.where(rowv == r, jnp.ones_like(vw), vw)
            d = jnp.dot(vw, p, preferred_element_type=F32)
            acc[rb] = d if cb == 0 else acc[rb] + d
            if cb == NC - 1:
                pend.append((t + EPI_LAG, rb, hb, qbb))
                mfin.pop(rb)

        def finish(t, force=False):
            for item in list(pend):
                if item[0] <= t or force:
                    pend.remove(item)
                    _, rb, hb_, qbb = item
                    ot_s[hb_, :, qcols(qbb)] = acc.pop(rb)

        pend = []
        for t in range(*(trange or (0, nsteps))):
            doB = t - LAG >= bmin
            if ORDER == 0:
                if doA:
                    stepA(t)
                if doB:
                    stepB(t)
            else:
                if doB:
                    stepB(t)
                if doA:
                    stepA(t)
            finish(t)
        finish(0, True)
        return mrun, mfin, acc

    assert U % 2 == 0 and 1 <= DELTA < NC
    make_qm(0, 0)
    if VR:
        for c in range(NC):
            make_kb(0, 0, c, range(DH))
    if not MERGE:
        st0 = run(0, U * NC, True, 0, ({}, {}, {}), True)

    def shift(st):
        mrun, mfin, acc = st
        assert set(mrun) == {U - 1} and set(mfin) == {U - 2} and set(acc) == {U - 2}, (mrun.keys(), mfin.keys(), acc.keys())
        return mrun[U - 1], mfin[U - 2], acc[U - 2]

    def unshift(c):
        return {-1: c[0]}, {-2: c[1]}, {-2: c[2]}

    def body(i, c):
        @pl.when(i == 2)
        def _():
            for cp in cps:
                cp.start()
        base = i * U
        return shift(run(base, U * NC, True, -LAG, unshift(c), True))

    with jax.named_scope("z3_attn_loop"):
        if MERGE:
            c0_ = (jnp.zeros((8, BQ), F32), jnp.zeros((1, BQ), F32), jnp.zeros((WIN, BQ), F32))
            c = lax.fori_loop(0, NIT // U, body, c0_)
        else:
            c = lax.fori_loop(1, NIT // U, body, shift(st0))
    for cp in cps:
        cp.wait()
    wot_s[...] = wo_s[...].T
    rowb = lax.broadcasted_iota(jnp.int32, (KP - D, 128), 0)
    for t in range(F // 128):
        brow = jnp.broadcast_to(b1_s[t:t + 1, :].astype(F32), (KP - D, 128))
        w1_s[D:, t * 128:(t + 1) * 128] = jnp.where(rowb == 0, brow, 0.0).astype(BF)

    ones_blk = (lax.broadcasted_iota(jnp.int32, (KP - D, TB3), 0) == 0).astype(F32)

    row8t = lax.broadcasted_iota(jnp.int32, (8, TB3), 0)

    def cols3(t):
        if isinstance(t, int):
            return slice(t * TB3, (t + 1) * TB3)
        return pl.ds(pl.multiple_of(t * TB3, TB3), TB3)

    def p3a(t, slot):
        cols = cols3(t)
        res = []
        for hh in range(H):
            win = (hh * DH // 8) * 8
            r = (hh * DH - win + DH) % WIN
            a = ot_s[hh, :, cols]
            res.append(a * pltpu.reciprocal(a[r:r + 1, :], full_range=False))
        blocks = []
        for v in range(D // 8):
            h0, h1 = (8 * v) // DH, (8 * v + 7) // DH
            w0 = (h0 * DH // 8) * 8
            blk = res[h0][8 * v - w0:8 * v - w0 + 8, :]
            if h1 != h0:
                w1 = (h1 * DH // 8) * 8
                blk = jnp.where(row8t < h1 * DH - 8 * v, blk, res[h1][8 * v - w1:8 * v - w1 + 8, :])
            blocks.append(blk)
        ot = jnp.concatenate(blocks, axis=0).astype(BF)
        attn = jnp.dot(wot_s[...], ot, preferred_element_type=F32)
        h = xt_s[:, cols].astype(F32) + attn
        h_s[slot] = h
        hn_s[slot] = jnp.concatenate([_ln_t(h), ones_blk], axis=0).astype(BF).T

    def ffn(t, slot):
        cols = cols3(t)
        hn = hn_s[slot]
        y = h_s[slot]
        for fc in range(F // FC):
            z = jnp.dot(hn, w1_s[:, fc * FC:(fc + 1) * FC], preferred_element_type=F32)
            sp = jnp.log1p(jnp.exp(-jnp.abs(z))) + jnp.maximum(z, 0.0)
            act = (z * jnp.tanh(sp)).astype(BF)
            y = y + lax.dot_general(w2t_s[:, fc * FC:(fc + 1) * FC], act, NT, preferred_element_type=F32)
        o_s[:, cols] = y.astype(o_s.dtype)

    st = unshift(c)
    for t in range(LAG):
        st = run(NIT, LAG, False, -LAG, st, False, (t, t + 1))
        if t == 0:
            p3a(0, 0)

    npair = S // (2 * TB3)

    def p3_body(i, _):
        t0 = 2 * i
        p3a(t0 + 1, 1)
        ffn(t0, 0)
        p3a(jnp.minimum(t0 + 2, S // TB3 - 1), 0)
        ffn(t0 + 1, 1)
        dcols = pl.ds(pl.multiple_of(t0 * TB3, 2 * TB3), 2 * TB3)
        pltpu.make_async_copy(o_s.at[:, dcols], out_hbm.at[:, dcols], sems.at[0]).start()
        return 0

    with jax.named_scope("z6_ffn_loop"):
        lax.fori_loop(0, npair, p3_body, 0)
    with jax.named_scope("z7_wait_out"):
        pltpu.make_async_copy(o_s, out_hbm, sems.at[0]).wait()


@jax.jit
def pallas_sequential_preLN__mha_block__dense_activation_mish__prompt_kernel(
    A_x, A_wqkv, A_wo, B_x, B_w1, B_b1, B_w2,
):
    del B_x
    xt = A_x.reshape(S, D).T
    w2t = B_w2.T
    b1 = B_b1.reshape(F // 128, 128)
    hbm = pl.BlockSpec(memory_space=pltpu.HBM)
    out_t = pl.pallas_call(
        _kernel,
        out_shape=jax.ShapeDtypeStruct((D, S), A_x.dtype),
        in_specs=[hbm] * 6,
        out_specs=hbm,
        scratch_shapes=[
            pltpu.VMEM((D, S), BF),
            pltpu.VMEM((D, 3 * D), BF),
            pltpu.VMEM((D, D), BF),
            pltpu.VMEM((2 * D, D), BF),
            pltpu.VMEM((D, S), BF),
            pltpu.VMEM((NG, 64, S), U32),
            pltpu.VMEM((NG, S, 128), F32),
            pltpu.VMEM((D, S), F32),
            pltpu.VMEM((H, WIN, S), F32),
            pltpu.VMEM((S, BQ), F32),
            pltpu.VMEM((S, BQ), F32),
            pltpu.VMEM((U, 64, BQ), U32),
            pltpu.VMEM((D, D), BF),
            pltpu.VMEM((D, D), BF),
            pltpu.VMEM((KP, F), BF),
            pltpu.VMEM((F // 128, 128), BF),
            pltpu.VMEM((D, F), BF),
            pltpu.VMEM((2, TB3, KP), BF),
            pltpu.VMEM((2, D, TB3), F32),
            pltpu.VMEM((D, S), BF),
            pltpu.VMEM((H, WIN, S), F32),
            pltpu.VMEM((U, DH, 8, BQ), F32),
            pltpu.VMEM((2, NC * max(VR // 8, 1), DH, 8, 128), F32),
            pltpu.SemaphoreType.DMA((13,)),
        ],
        compiler_params=pltpu.CompilerParams(vmem_limit_bytes=120 * 1024 * 1024),
    )(xt, A_wqkv, A_wo, B_w1, b1, w2t)
    return out_t.T.reshape(1, S, D)
```
